```python
import jax
import jax.numpy as jnp

def _softmax(x, axis=-1):
    return jax.nn.softmax(x, axis=axis)
def _gelu(x):
    return jax.nn.gelu(x, approximate=True)
def _silu(x):
    return jax.nn.silu(x)
def _sigmoid(x):
    return jax.nn.sigmoid(x)
def _layernorm(x, axis=-1, eps=1e-5):
    m = jnp.mean(x, axis=axis, keepdims=True)
    v = jnp.var(x, axis=axis, keepdims=True)
    return (x - m) / jnp.sqrt(v + eps)
def _scatter_add(tgt, idx, src, axis=0):
    return tgt.at[idx].add(src)
def _segment_sum(src, seg, n):
    return jax.ops.segment_sum(src, seg, n)
class _Rng:
    def __init__(self, key):
        self._k = key
    def _next(self):
        self._k, sub = jax.random.split(self._k)
        return sub
    def normal(self, shape):
        return jax.random.normal(self._next(), shape, dtype=jnp.bfloat16)
    def randint(self, lo, hi, shape):
        return jax.random.randint(self._next(), shape, lo, hi, dtype=jnp.int32)
    def uniform(self, shape, lo=0.0, hi=1.0):
        return jax.random.uniform(self._next(), shape, jnp.bfloat16, lo, hi)
    def permutation(self, n):
        return jax.random.permutation(self._next(), n)


kernel_name = 'parallel_sum__sliding_block_cached__glu_gated_swiglu__decode'

def setup_inputs():
    _rng = _Rng(jax.random.key(int.from_bytes(__import__("os").urandom(4), "little")))
    _w = (lambda a: (lambda t: t.astype(jnp.bfloat16) if jnp.issubdtype(t.dtype, jnp.floating) else t)(jnp.asarray(a)))
    def _A_setup():
        B, Sq, D = 4, 1, 640
        Hq, Hkv, Sk, Dh = 32, 32, 8192, 192
        assert Hq % Hkv == 0, (Hq, Hkv)
        return {
            "x": _w((lambda *s: _rng.normal(s) * 0.05)(B, Sq, D)),
            "k_cache": _w((lambda *s: _rng.normal(s) * 0.05)(B, Hkv, Sk, Dh)),
            "v_cache": _w((lambda *s: _rng.normal(s) * 0.05)(B, Hkv, Sk, Dh)),
            "wq": _w((lambda *s: _rng.normal(s) * 0.05)(D, Hq * Dh) * (D ** -0.5)),
            "wo": _w((lambda *s: _rng.normal(s) * 0.05)(Hq * Dh, D) * ((Hq * Dh) ** -0.5)),
        }
    _A_in = _A_setup()

    def _B_setup():
        B, S, D, F = 4, 1, 640, 1536
        return {
            "x": _w((lambda *s: _rng.normal(s) * 0.05)(B, S, D)),
            "w1": _w((lambda *s: _rng.normal(s) * 0.05)(D, F) * (2.0 / D) ** 0.5),
            "w3": _w((lambda *s: _rng.normal(s) * 0.05)(D, F) * (2.0 / D) ** 0.5),
            "w2": _w((lambda *s: _rng.normal(s) * 0.05)(F, D) * (2.0 / F) ** 0.5),
        }
    _B_in = _B_setup()

    return {
        "A_x": _A_in["x"],
        "A_k_cache": _A_in["k_cache"],
        "A_v_cache": _A_in["v_cache"],
        "A_wq": _A_in["wq"],
        "A_wo": _A_in["wo"],
        "B_x": _B_in["x"],
        "B_w1": _B_in["w1"],
        "B_w3": _B_in["w3"],
        "B_w2": _B_in["w2"],
    }

def reference(A_x, A_k_cache, A_v_cache, A_wq, A_wo, B_x, B_w1, B_w3, B_w2):
    def _A_ref(x, k_cache, v_cache, wq, wo):
        B, Sq, D = x.shape
        Hq, Dh = 32, 192
        Hkv, Sk = k_cache.shape[1], k_cache.shape[2]
        W = min(4096, max(256, Sk // 4))
        rep = Hq // Hkv
        q = (lambda x, *d: x.transpose(*d))((x @ wq).reshape(B, Sq, Hq, Dh), 0, 2, 1, 3)
        k = jnp.repeat(k_cache[:, :, Sk - W:, :], rep, axis=1)
        v = jnp.repeat(v_cache[:, :, Sk - W:, :], rep, axis=1)
        scores = jnp.einsum("bhqd,bhkd->bhqk", q, k) * (Dh ** -0.5)
        p = _softmax(scores, axis=-1)
        o = jnp.einsum("bhqk,bhkd->bhqd", p, v)
        return (lambda x, *d: x.transpose(*d))(o, 0, 2, 1, 3).reshape(B, Sq, Hq * Dh) @ wo

    def _B_ref(x, w1, w3, w2):
        gate = jnp.einsum("bsd,df->bsf", x, w1)
        up = jnp.einsum("bsd,df->bsf", x, w3)
        h = _silu(gate) * up
        out = jnp.einsum("bsf,fd->bsd", h, w2)
        return out

    x = A_x
    xn = _layernorm(x, axis=-1)
    return x + _A_ref(xn, A_k_cache, A_v_cache, A_wq, A_wo) + _B_ref(xn, B_w1, B_w3, B_w2)
```

```python
import jax
import jax.numpy as jnp
import jax.experimental.pallas as pl
import jax.experimental.pallas.tpu as pltpu

_HQ = 32
_DH = 192
_NBUF = 8


def _kernel(x_hbm, kt_hbm, vt_hbm, wq_hbm, wo_hbm, w1_hbm, w3_hbm, w2_hbm,
            out_ref,
            x_v, wq_v, wo_v, w1_v, w3_v, w2_v, kbuf, vbuf, q_s,
            sem_w, sem_k, sem_v, *, B, H, rep, Sk, W):
    f32, bf16 = jnp.float32, jnp.bfloat16
    n_chunks = H * B
    start = Sk - W

    def kv_copies(i, slot):
        b = i % B
        hk = (i // B) // rep
        return (
            pltpu.make_async_copy(kt_hbm.at[b, hk, :, pl.ds(start, W)], kbuf.at[slot], sem_k.at[slot]),
            pltpu.make_async_copy(vt_hbm.at[b, hk, :, pl.ds(start, W)], vbuf.at[slot], sem_v.at[slot]),
        )

    def kv_start(i, slot):
        ck, cv = kv_copies(i, slot)
        ck.start(priority=0)
        cv.start(priority=1)

    c_x = pltpu.make_async_copy(x_hbm, x_v, sem_w.at[0])
    c_wq = pltpu.make_async_copy(wq_hbm, wq_v, sem_w.at[1])
    c_w1 = pltpu.make_async_copy(w1_hbm, w1_v, sem_w.at[2])
    c_w3 = pltpu.make_async_copy(w3_hbm, w3_v, sem_w.at[3])
    c_w2 = pltpu.make_async_copy(w2_hbm, w2_v, sem_w.at[4])
    c_wo = pltpu.make_async_copy(wo_hbm, wo_v, sem_w.at[5])

    c_x.start()
    c_wq.start()
    for i in range(_NBUF):
        kv_start(i, i)
    c_wo.start()
    c_w1.start()
    c_w3.start()
    c_w2.start()

    c_x.wait()
    x = x_v[...].astype(f32)
    mu = jnp.mean(x, axis=-1, keepdims=True)
    xc = x - mu
    var = jnp.mean(xc * xc, axis=-1, keepdims=True)
    xn = (xc / jnp.sqrt(var + 1e-5)).astype(bf16)

    c_wq.wait()
    q = jnp.dot(xn, wq_v[...], preferred_element_type=f32)
    for h in range(H):
        q_s[h] = q[:, h * _DH:(h + 1) * _DH].astype(bf16)

    c_wo.wait()
    scale = _DH ** -0.5
    row_s = jax.lax.broadcasted_iota(jnp.int32, (B, W), 0)
    row_o = jax.lax.broadcasted_iota(jnp.int32, (B, _DH), 0)

    def head_body(h, acc):
        qh = q_s[h]
        s = jnp.zeros((B, W), f32)
        for b in range(B):
            i = h * B + b
            slot = i % _NBUF
            kv_copies(i, slot)[0].wait()
            sb = jnp.dot(qh, kbuf[slot], preferred_element_type=f32)
            s = jnp.where(row_s == b, sb, s)
        s = s * scale
        m = jnp.max(s, axis=-1, keepdims=True)
        p = jnp.exp(s - m)
        l = jnp.sum(p, axis=-1, keepdims=True)
        pb = p.astype(bf16)
        o = jnp.zeros((B, _DH), f32)
        for b in range(B):
            i = h * B + b
            slot = i % _NBUF
            kv_copies(i, slot)[1].wait()
            ob = jax.lax.dot_general(pb, vbuf[slot], (((1,), (1,)), ((), ())),
                                     preferred_element_type=f32)
            o = jnp.where(row_o == b, ob, o)

            @pl.when(i + _NBUF < n_chunks)
            def _():
                kv_start(i + _NBUF, slot)
        o = (o / l).astype(bf16)
        woh = wo_v[pl.ds(pl.multiple_of(h * _DH, _DH), _DH), :]
        return acc + jnp.dot(o, woh, preferred_element_type=f32)

    c_w1.wait()
    c_w3.wait()
    g = jnp.dot(xn, w1_v[...], preferred_element_type=f32)
    u = jnp.dot(xn, w3_v[...], preferred_element_type=f32)
    hid = (g * jax.nn.sigmoid(g) * u).astype(bf16)
    c_w2.wait()
    ffn = jnp.dot(hid, w2_v[...], preferred_element_type=f32)

    acc = jax.lax.fori_loop(0, H, head_body, x + ffn)
    out_ref[...] = acc.astype(out_ref.dtype)


@jax.jit
def pallas_parallel_sum__sliding_block_cached__glu_gated_swiglu__decode_kernel(
    A_x: jax.Array,
    A_k_cache: jax.Array,
    A_v_cache: jax.Array,
    A_wq: jax.Array,
    A_wo: jax.Array,
    B_x: jax.Array,
    B_w1: jax.Array,
    B_w3: jax.Array,
    B_w2: jax.Array,
):
    del B_x
    B, Sq, D = A_x.shape
    assert Sq == 1
    Hkv, Sk = A_k_cache.shape[1], A_k_cache.shape[2]
    W = min(4096, max(256, Sk // 4))
    F = B_w1.shape[1]
    dt = A_x.dtype

    kt = jnp.swapaxes(A_k_cache, 2, 3)
    vt = jnp.swapaxes(A_v_cache, 2, 3)
    x2 = A_x.reshape(B, D)

    def kern(*refs):
        _kernel(*refs, B=B, H=_HQ, rep=_HQ // Hkv, Sk=Sk, W=W)

    out = pl.pallas_call(
        kern,
        out_shape=jax.ShapeDtypeStruct((B, D), dt),
        in_specs=[pl.BlockSpec(memory_space=pl.ANY)] * 8,
        out_specs=pl.BlockSpec(memory_space=pltpu.VMEM),
        scratch_shapes=[
            pltpu.VMEM((B, D), dt),
            pltpu.VMEM((D, _HQ * _DH), A_wq.dtype),
            pltpu.VMEM((_HQ * _DH, D), A_wo.dtype),
            pltpu.VMEM((D, F), B_w1.dtype),
            pltpu.VMEM((D, F), B_w3.dtype),
            pltpu.VMEM((F, D), B_w2.dtype),
            pltpu.VMEM((_NBUF, _DH, W), A_k_cache.dtype),
            pltpu.VMEM((_NBUF, _DH, W), A_v_cache.dtype),
            pltpu.VMEM((_HQ, B, _DH), dt),
            pltpu.SemaphoreType.DMA((6,)),
            pltpu.SemaphoreType.DMA((_NBUF,)),
            pltpu.SemaphoreType.DMA((_NBUF,)),
        ],
        compiler_params=pltpu.CompilerParams(vmem_limit_bytes=96 * 2**20),
    )(x2, kt, vt, A_wq, A_wo, B_w1, B_w3, B_w2)
    return out.reshape(B, Sq, D)
```

```python
import jax
import jax.numpy as jnp
import jax.experimental.pallas as pl
import jax.experimental.pallas.tpu as pltpu

_HQ = 32
_DH = 192
_PC = 128
_PW = 128
_NBUF = 5


def _kernel(x_hbm, kt_hbm, vt_hbm, wq_hbm, wo_hbm, w1_hbm, w3_hbm, w2_hbm,
            out_ref,
            x_v, wq_v, wo_v, w1_v, w3_v, w2_v, kbuf, vbuf, q_s,
            sem_w, sem_k, sem_v, *, B, H, rep, Sk, W):
    f32, bf16 = jnp.float32, jnp.bfloat16
    n_chunks = H * B
    start = Sk - W

    def kv_start(t, i, slot):
        src, dst, sem = ((kt_hbm, kbuf, sem_k), (vt_hbm, vbuf, sem_v))[t]
        b = i % B
        hk = (i // B) // rep
        for c in range(W // _PC):
            pltpu.make_async_copy(
                src.at[b, hk, :, pl.ds(start + c * _PC, _PC)],
                dst.at[slot, :, pl.ds(c * _PC, _PC)],
                sem.at[slot]).start(priority=(c + t) % 2)

    def kv_wait(t, slot):
        dst, sem = ((kbuf, sem_k), (vbuf, sem_v))[t]
        pltpu.make_async_copy(dst.at[slot], dst.at[slot], sem.at[slot]).wait()

    def w_start(src, dst, sem, axis):
        n = src.shape[axis] // _PW
        for c in range(n):
            idx = (slice(None), pl.ds(c * _PW, _PW)) if axis else (pl.ds(c * _PW, _PW), slice(None))
            pltpu.make_async_copy(src.at[idx], dst.at[idx], sem).start(priority=c % 2)
        return pltpu.make_async_copy(dst, dst, sem)

    c_x = pltpu.make_async_copy(x_hbm, x_v, sem_w.at[0])
    c_x.start()
    c_wq = w_start(wq_hbm, wq_v, sem_w.at[1], 1)
    c_w1 = w_start(w1_hbm, w1_v, sem_w.at[2], 1)
    c_w3 = w_start(w3_hbm, w3_v, sem_w.at[3], 1)
    c_w2 = w_start(w2_hbm, w2_v, sem_w.at[4], 0)
    c_wo = w_start(wo_hbm, wo_v, sem_w.at[5], 0)
    for i in range(_NBUF):
        kv_start(0, i, i)
        kv_start(1, i, i)

    c_x.wait()
    x = x_v[...].astype(f32)
    mu = jnp.mean(x, axis=-1, keepdims=True)
    xc = x - mu
    var = jnp.mean(xc * xc, axis=-1, keepdims=True)
    xn = (xc / jnp.sqrt(var + 1e-5)).astype(bf16)

    c_wq.wait()
    q = jnp.dot(xn, wq_v[...], preferred_element_type=f32)
    for h in range(H):
        q_s[h] = q[:, h * _DH:(h + 1) * _DH].astype(bf16)

    scale = _DH ** -0.5
    row_s = jax.lax.broadcasted_iota(jnp.int32, (B, W), 0)
    row_o = jax.lax.broadcasted_iota(jnp.int32, (B, _DH), 0)

    def head_body(h, acc):
        qh = q_s[h]
        s = jnp.zeros((B, W), f32)
        for b in range(B):
            i = h * B + b
            slot = i % _NBUF
            kv_wait(0, slot)
            sb = jnp.dot(qh, kbuf[slot], preferred_element_type=f32)
            s = jnp.where(row_s == b, sb, s)

            @pl.when(i + _NBUF < n_chunks)
            def _():
                kv_start(0, i + _NBUF, slot)
        s = s * scale
        m = jnp.max(s, axis=-1, keepdims=True)
        p = jnp.exp(s - m)
        l = jnp.sum(p, axis=-1, keepdims=True)
        pb = p.astype(bf16)
        o = jnp.zeros((B, _DH), f32)
        for b in range(B):
            i = h * B + b
            slot = i % _NBUF
            kv_wait(1, slot)
            ob = jax.lax.dot_general(pb, vbuf[slot], (((1,), (1,)), ((), ())),
                                     preferred_element_type=f32)
            o = jnp.where(row_o == b, ob, o)

            @pl.when(i + _NBUF < n_chunks)
            def _():
                kv_start(1, i + _NBUF, slot)
        o = (o / l).astype(bf16)
        woh = wo_v[pl.ds(pl.multiple_of(h * _DH, _DH), _DH), :]
        return acc + jnp.dot(o, woh, preferred_element_type=f32)

    c_w1.wait()
    c_w3.wait()
    g = jnp.dot(xn, w1_v[...], preferred_element_type=f32)
    u = jnp.dot(xn, w3_v[...], preferred_element_type=f32)
    hid = (g * jax.nn.sigmoid(g) * u).astype(bf16)
    c_w2.wait()
    ffn = jnp.dot(hid, w2_v[...], preferred_element_type=f32)

    c_wo.wait()
    acc = jax.lax.fori_loop(0, H, head_body, x + ffn)
    out_ref[...] = acc.astype(out_ref.dtype)


@jax.jit
def pallas_parallel_sum__sliding_block_cached__glu_gated_swiglu__decode_kernel(
    A_x: jax.Array,
    A_k_cache: jax.Array,
    A_v_cache: jax.Array,
    A_wq: jax.Array,
    A_wo: jax.Array,
    B_x: jax.Array,
    B_w1: jax.Array,
    B_w3: jax.Array,
    B_w2: jax.Array,
):
    del B_x
    B, Sq, D = A_x.shape
    assert Sq == 1
    Hkv, Sk = A_k_cache.shape[1], A_k_cache.shape[2]
    W = min(4096, max(256, Sk // 4))
    F = B_w1.shape[1]
    dt = A_x.dtype

    kt = jnp.swapaxes(A_k_cache, 2, 3)
    vt = jnp.swapaxes(A_v_cache, 2, 3)
    x2 = A_x.reshape(B, D)

    def kern(*refs):
        _kernel(*refs, B=B, H=_HQ, rep=_HQ // Hkv, Sk=Sk, W=W)

    out = pl.pallas_call(
        kern,
        out_shape=jax.ShapeDtypeStruct((B, D), dt),
        in_specs=[pl.BlockSpec(memory_space=pl.ANY)] * 8,
        out_specs=pl.BlockSpec(memory_space=pltpu.VMEM),
        scratch_shapes=[
            pltpu.VMEM((B, D), dt),
            pltpu.VMEM((D, _HQ * _DH), A_wq.dtype),
            pltpu.VMEM((_HQ * _DH, D), A_wo.dtype),
            pltpu.VMEM((D, F), B_w1.dtype),
            pltpu.VMEM((D, F), B_w3.dtype),
            pltpu.VMEM((F, D), B_w2.dtype),
            pltpu.VMEM((_NBUF, _DH, W), A_k_cache.dtype),
            pltpu.VMEM((_NBUF, _DH, W), A_v_cache.dtype),
            pltpu.VMEM((_HQ, B, _DH), dt),
            pltpu.SemaphoreType.DMA((6,)),
            pltpu.SemaphoreType.DMA((_NBUF,)),
            pltpu.SemaphoreType.DMA((_NBUF,)),
        ],
        compiler_params=pltpu.CompilerParams(vmem_limit_bytes=96 * 2**20),
    )(x2, kt, vt, A_wq, A_wo, B_w1, B_w3, B_w2)
    return out.reshape(B, Sq, D)
```
